```python
import os as _os
_os.environ.setdefault('JAX_PLATFORMS', 'cpu')
import jax
import jax.numpy as jnp

def _softmax(x, axis=-1):
    return jax.nn.softmax(x, axis=axis)

def _gelu(x):
    return jax.nn.gelu(x, approximate=True)

def _silu(x):
    return jax.nn.silu(x)

def _sigmoid(x):
    return jax.nn.sigmoid(x)

def _layernorm(x, axis=-1, eps=1e-05):
    m = jnp.mean(x, axis=axis, keepdims=True)
    v = jnp.var(x, axis=axis, keepdims=True)
    return (x - m) / jnp.sqrt(v + eps)

def _scatter_add(tgt, idx, src, axis=0):
    return tgt.at[idx].add(src)

def _segment_sum(src, seg, n):
    return jax.ops.segment_sum(src, seg, n)

class _Rng:

    def __init__(self, key):
        self._k = key

    def _next(self):
        self._k, sub = jax.random.split(self._k)
        return sub

    def normal(self, shape):
        return jax.random.normal(self._next(), shape, dtype=jnp.bfloat16)

    def randint(self, lo, hi, shape):
        return jax.random.randint(self._next(), shape, lo, hi, dtype=jnp.int32)

    def uniform(self, shape, lo=0.0, hi=1.0):
        return jax.random.uniform(self._next(), shape, jnp.bfloat16, lo, hi)

    def permutation(self, n):
        return jax.random.permutation(self._next(), n)
kernel_name = 'sequential_preLN__memory_aug_recurrent_mem_tr__mixer_token_mlp__prompt'

def setup_inputs():
    _rng = _Rng(jax.random.key(int.from_bytes(__import__("os").urandom(4), "little")))
    _w = lambda a: (lambda t: t.astype(jnp.bfloat16) if jnp.issubdtype(t.dtype, jnp.floating) else t)(jnp.asarray(a))

    def _A_setup():
        B, S, Dm = (1, 2048, 448)
        H, Dh = (16, 256)
        M, seg = (8, 32)
        seg = min(seg, S)
        S = S // seg * seg
        return {'x': _w((lambda *s: _rng.normal(s) * 0.05)(B, S, Dm)), 'mem0': _w((lambda *s: _rng.normal(s) * 0.2)(B, M, Dm)), 'Wq': _w((lambda *s: _rng.normal(s) * 1.6)(Dm, H, Dh) * Dm ** (-0.5)), 'Wk': _w((lambda *s: _rng.normal(s) * 1.6)(Dm, H, Dh) * Dm ** (-0.5)), 'Wv': _w((lambda *s: _rng.normal(s) * 0.2)(Dm, H, Dh) * Dm ** (-0.5)), 'Wo': _w((lambda *s: _rng.normal(s) * 0.2)(H, Dh, Dm) * (H * Dh) ** (-0.5)), 'seg_len': seg}
    _A_in = _A_setup()

    def _B_setup():
        B, S, D, F = (1, 2048, 448, 1792)
        return {'x': _w((lambda *s: _rng.normal(s) * 0.05)(B, S, D)), 'w1': _w((lambda *s: _rng.normal(s) * 0.2)(S, F) * S ** (-0.5)), 'b1': _w((lambda *s: _rng.normal(s) * 0.2)(F) * 0.02), 'w2': _w((lambda *s: _rng.normal(s) * 0.2)(F, S) * F ** (-0.5)), 'b2': _w((lambda *s: _rng.normal(s) * 0.05)(S) * 0.02)}
    _B_in = _B_setup()
    return {'A_x': _A_in['x'], 'A_mem0': _A_in['mem0'], 'A_Wq': _A_in['Wq'], 'A_Wk': _A_in['Wk'], 'A_Wv': _A_in['Wv'], 'A_Wo': _A_in['Wo'], 'A_seg_len': _A_in['seg_len'], 'B_x': _B_in['x'], 'B_w1': _B_in['w1'], 'B_b1': _B_in['b1'], 'B_w2': _B_in['w2'], 'B_b2': _B_in['b2']}

def reference(A_x, A_mem0, A_Wq, A_Wk, A_Wv, A_Wo, A_seg_len, B_x, B_w1, B_b1, B_w2, B_b2):

    def _A_ref(x, mem0, Wq, Wk, Wv, Wo, seg_len):
        B, S, Dm = x.shape
        H, Dh = (Wq.shape[1], Wq.shape[2])
        M = mem0.shape[1]
        scale = Dh ** (-0.5)
        n_seg = S // seg_len
        L = M + seg_len
        idx = jnp.arange(L)
        mask = (idx[:, None] < M) | (idx[:, None] >= idx[None, :])
        mem = mem0
        outs = []
        for s in range(n_seg):
            xs = x[:, s * seg_len:(s + 1) * seg_len, :].copy()
            h = jnp.concatenate([mem, xs], axis=1)
            q = jnp.einsum('btd,dhe->bhte', h, Wq)
            k = jnp.einsum('btd,dhe->bhte', h, Wk)
            v = jnp.einsum('btd,dhe->bhte', h, Wv)
            scores = jnp.einsum('bhqe,bhke->bhqk', q, k) * scale
            scores = jnp.where(mask[None, None], scores, -1000000000.0)
            p = _softmax(scores, axis=-1)
            o = jnp.einsum('bhqk,bhke->bhqe', p, v)
            o = jnp.einsum('bhte,hed->btd', o, Wo)
            mem = o[:, :M, :].copy()
            outs.append(o[:, M:, :])
        return jnp.concatenate(outs, axis=1)

    def _B_ref(x, w1, b1, w2, b2):
        B, S, D = x.shape
        h = _layernorm(x, axis=-1)
        u = jnp.einsum('bsd,sf->bdf', h, w1) + b1
        u = _gelu(u)
        y = jnp.einsum('bdf,fs->bds', u, w2) + b2
        return (lambda x, *d: x.transpose(*d))(y, 0, 2, 1)
    x = A_x
    h = x + _A_ref(_layernorm(x, axis=-1), A_mem0, A_Wq, A_Wk, A_Wv, A_Wo, A_seg_len)
    h2 = h + _B_ref(_layernorm(h, axis=-1), B_w1, B_b1, B_w2, B_b2)
    return h2
```

```python
import jax
import jax.numpy as jnp
from jax import lax
import jax.experimental.pallas as pl
import jax.experimental.pallas.tpu as pltpu

F32 = jnp.float32
BF16 = jnp.bfloat16
U32 = jnp.uint32

S, D, DP, H, E, M, SEG, F = 2048, 448, 512, 16, 256, 8, 32, 1792
DA = 384
L = M + SEG
NG = L // 8
NB = S // 128
NP = H // 2
PW = 2 * D
EPS = 1e-5
SCOPES = False
DEPTH = 3
CAUSAL = True
ONLY_LOOP = False
XPOSE = False
STEPS = 4
FLAGS = None
STORE = ''
ORDER = "U T0 C0 T1 C1 T2 C2 T3 C3 T4 C4 T5 T6 T7 V0 D0 V1 D1 X0 V2 D2 X1 V3 D3 X2 V4 D4 X3 V5 X4 V6 V7 M0 P A M1"


def _scope(name):
    import contextlib
    return jax.named_scope(name) if SCOPES else contextlib.nullcontext()


_NN = (((1,), (0,)), ((), ()))
_NT = (((1,), (1,)), ((), ()))
dot_W = lambda a, b: lax.dot_general(a, b, _NT, preferred_element_type=F32)
dot_T = lambda a, b: lax.dot_general(a, b, _NN, preferred_element_type=F32)
dot_U = lambda a, b: lax.dot_general(a, b, _NN, preferred_element_type=F32)
dot_S1 = lambda a, b: lax.dot_general(a, b, _NN if XPOSE else _NT, preferred_element_type=F32)
dot_S2 = lambda a, b: lax.dot_general(a, b, _NN if XPOSE else _NT, preferred_element_type=F32)
dot_Z = lambda a, b: lax.dot_general(a, b, _NN, preferred_element_type=F32)
dot_AF = lambda a, b: lax.dot_general(a, b, _NN, preferred_element_type=F32)
dot_PV = lambda a, b: lax.dot_general(a, b, _NN, preferred_element_type=F32)
dot_MX = lambda a, b: lax.dot_general(a, b, _NN, preferred_element_type=F32)
dot_Y = lambda a, b: lax.dot_general(a, b, _NN, preferred_element_type=F32)


def _ln_rows(x):
    m = jnp.mean(x, axis=0, keepdims=True)
    c = x - m
    v = jnp.mean(c * c, axis=0, keepdims=True)
    return c * lax.rsqrt(v + EPS)


def _lanes(rows):
    return lax.broadcasted_iota(jnp.int32, (rows, 128), 1)


def _swap8(v):
    lane = _lanes(8)
    sub = lax.broadcasted_iota(jnp.int32, (8, 128), 0)
    v = pltpu.roll(v, 0, 1, stride=1, stride_axis=0)
    v = jnp.take_along_axis(v, (sub + lane + 1) & 7, axis=0)
    v = pltpu.roll(v, 121, 1, stride=1, stride_axis=0)
    return jnp.take_along_axis(v, 7 - sub, axis=0)


def _aligned(i, n):
    return i * n if isinstance(i, int) else pl.multiple_of(i * n, n)


def _kernel(xT_hbm, mem_ref, wq_hbm, wk_hbm, wv_hbm, woT_hbm, w1_hbm, b1_ref, w2_hbm, b2_ref,
            out_hbm,
            wraw, woT, xT, wt, wu, wv, wz, xn, w1, w2, tt, ut, vt, cs, ps, zb, onat, hT, hnT, u, ostage,
            wsem, xsem, msem, osem):
    def raw_copy(n, w, p):
        return pltpu.make_async_copy(w.bitcast(U32).at[:, p, :], wraw.at[n, p], wsem.at[n, p])

    def a_copies(p):
        return [raw_copy(0, wq_hbm, p), raw_copy(1, wk_hbm, p)]

    def b_copies(p):
        return [raw_copy(2, wv_hbm, p),
                pltpu.make_async_copy(woT_hbm.at[pl.ds(2 * p, 2)], woT.at[pl.ds(2 * p, 2)], wsem.at[3, p])]

    def x_copy(b):
        return pltpu.make_async_copy(xT_hbm.at[:, pl.ds(_aligned(b, 128), 128)], xT.at[b], xsem.at[b])

    def w1_copy(b):
        rows = pl.ds(_aligned(b, 128), 128)
        return pltpu.make_async_copy(w1_hbm.at[rows], w1.at[rows], msem.at[0, b])

    def w2_copy(b):
        rows = pl.ds(_aligned(b, F // NB), F // NB)
        return pltpu.make_async_copy(w2_hbm.at[rows], w2.at[rows], msem.at[1, b])

    def head_pair(n, p):
        words = wraw[n, p]
        even = pltpu.bitcast(words << 16, F32)
        odd = pltpu.bitcast(words & jnp.uint32(0xFFFF0000), F32)
        return even, odd

    def shared_tile(l0, l1, r0, r1):
        rb = jnp.concatenate([r0[DA:D], r1[DA:D]], axis=0).astype(BF16)
        return jnp.where(_lanes(l0.shape[0]) < 64, dot_W(l0, rb), dot_W(l1, rb))

    def words(x):
        return pltpu.bitcast(x.astype(BF16), U32)

    def prep_x(b):
        n = _ln_rows(xT[b].astype(F32))
        n = jnp.concatenate([n, n[DA:D]], axis=0)
        for c in range(4):
            xn[pl.ds(_aligned(b, 128), 128), 128 * c:128 * (c + 1)] = n[128 * c:128 * (c + 1)].T

    def absorb_a(p):
        scale = E ** -0.5
        q0, q1 = head_pair(0, p)
        k0, k1 = head_pair(1, p)
        full = jnp.concatenate(
            [dot_W(q0[:DA], k0[:DA].astype(BF16)), dot_W(q1[:DA], k1[:DA].astype(BF16)),
             shared_tile(q0[:DA], q1[:DA], k0, k1)], axis=1)
        wt[p] = words(full * scale)
        wu[p] = words(shared_tile(k0, k1, q0, q1) * scale)

    def absorb_b(p):
        v0, v1 = head_pair(2, p)
        o0, o1 = woT[2 * p], woT[2 * p + 1]
        b0, b1, bs = dot_W(v0, o0[:DA]), dot_W(v1, o1[:DA]), shared_tile(v0, v1, o0, o1)
        wv[p] = words(jnp.concatenate([b0[:DA], b1[:DA], bs[:DA]], axis=1))
        low = _lanes(D - DA) < 64
        z0 = jnp.concatenate([b0[DA:], jnp.where(low, bs[DA:], 0.0)], axis=1)
        z1 = jnp.concatenate([b1[DA:], jnp.where(low, 0.0, bs[DA:])], axis=1)
        for dg in range(8):
            rows = slice(8 * dg, 8 * dg + 8)
            wz[dg, pl.ds(_aligned(p, 8), 8), :] = words(jnp.concatenate([z0[rows], z1[rows]], axis=0))

    if not ONLY_LOOP:
        queue = [a_copies(p) for p in range(NP)] + [b_copies(p) for p in range(NP)]
        queue[NP] = queue[NP] + [x_copy(0)]
        queue = queue + [[x_copy(1)]]
        for group in queue[:DEPTH]:
            for c in group:
                c.start()

        def phase(first, absorb):
            def body(p, carry):
                for i in range(NP):
                    @pl.when(p == i)
                    def _():
                        for c in queue[first + i]:
                            c.wait()
                        if first + i + DEPTH < len(queue):
                            for c in queue[first + i + DEPTH]:
                                c.start()
                with _scope("absorb"):
                    absorb(p)
                return carry
            lax.fori_loop(0, NP, body, 0)

        phase(0, absorb_a)
        phase(NP, absorb_b)
    prep_x(0)
    u[...] = jnp.broadcast_to(b1_ref[...].astype(F32).reshape(1, F), (D, F))

    def grp(x, g):
        return x[8 * g:8 * (g + 1)]

    def put_pair(dst, even, odd, p):
        for g in range(NG):
            dst(g)[pl.ds(16 * p, 16), :] = jnp.concatenate([grp(even, g), grp(odd, g)], axis=0).astype(BF16)

    def project(h, w_ref, dst, p):
        t = dot_T(h[:, :DA], pltpu.bitcast(w_ref[p], BF16))
        for c in range(3):
            put_pair(lambda g: dst.at[g, c], t[:, 128 * c:128 * (c + 1)], t[:, DA + 128 * c:DA + 128 * (c + 1)], p)
        tb = t[:, 2 * DA:]
        low = _lanes(L) < 64
        put_pair(lambda g: dst.at[g, 3], jnp.where(low, tb, 0.0), jnp.where(low, 0.0, tb), p)

    def visible(gq, gk):
        return (not CAUSAL) or gq == 0 or gk <= gq

    def step(mem, seg, mix):
        h = jnp.concatenate([mem, xn[pl.ds(_aligned(seg, SEG), SEG), :]], axis=0)
        hb = h[:, DA:]
        hbT = jnp.concatenate([hb, jnp.zeros((128 - L, 128), F32)], axis=0).T[:D - DA]
        cross, direct, probs, zs = {}, {}, {}, {}
        rows = [None] * NG

        def accumulate(g, v):
            rows[g] = v if rows[g] is None else rows[g] + v

        def op_U(p):
            t = dot_U(h[:, :D], pltpu.bitcast(wu[p], BF16))
            low = _lanes(L) < 64
            put_pair(lambda g: ut.at[g], jnp.where(low, t, 0.0), jnp.where(low, 0.0, t), p)

        def op_T(p):
            project(h, wt, tt, p)

        def op_V(p):
            project(h, wv, vt, p)

        def op_C(gk):
            gqs = [gq for gq in range(NG) if visible(gq, gk)]
            s = dot_S2(jnp.concatenate([grp(hb, gq) for gq in gqs], axis=0), ut[gk].T if XPOSE else ut[gk])
            for i, gq in enumerate(gqs):
                if 'c' in STORE:
                    cs[gq, 8 * gk:8 * gk + 8, :] = _swap8(grp(s, i))
                else:
                    cross[gq, gk] = _swap8(grp(s, i))

        def op_D(gq):
            n = sum(visible(gq, gk) for gk in range(NG))
            if XPOSE:
                keys = jnp.concatenate([tt[gq, c].T for c in range(4)], axis=0)
            else:
                keys = jnp.concatenate([tt[gq, c] for c in range(4)], axis=1)
            direct[gq] = dot_S1(h[:8 * n], keys)

        def op_X(gq):
            n = direct[gq].shape[0] // 8
            parts = []
            for gk in range(n):
                s = grp(direct[gq], gk) + (cs[gq, 8 * gk:8 * gk + 8, :] if 'c' in STORE else cross[gq, gk])
                if gq > 0 and gk == gq:
                    sub = lax.broadcasted_iota(jnp.int32, (8, 128), 0)
                    s = jnp.where(sub <= (_lanes(8) & 7), s, -1e9)
                elif gq > 0 and gk > gq:
                    s = jnp.full((8, 128), -1e9, F32)
                parts.append(s)
            s = jnp.concatenate(parts, axis=0)
            e = jnp.exp(s - jnp.max(s, axis=0, keepdims=True))
            pt = e * (1.0 / jnp.sum(e, axis=0, keepdims=True))
            for gk in range(n):
                if 'p' in STORE:
                    ps[gk, 8 * gq:8 * gq + 8, :] = _swap8(grp(pt, gk))
                else:
                    probs[gq, gk] = _swap8(grp(pt, gk))
            if n % 2:
                pt = jnp.concatenate([pt, jnp.zeros((8, 128), F32)], axis=0)
            zT = dot_Z(hbT[:, :pt.shape[0]], pt.astype(BF16))
            if 'z' in STORE:
                for dg in range(8):
                    zb[dg, 8 * gq:8 * gq + 8, :] = _swap8(grp(zT, dg))
            else:
                zs[gq] = [_swap8(grp(zT, dg)) for dg in range(8)]

        def op_A(dg):
            z = zb[dg] if 'z' in STORE else jnp.concatenate([zs[g][dg] for g in range(NG)], axis=0)
            part = dot_AF(z, pltpu.bitcast(wz[dg], BF16))
            for g in range(NG):
                accumulate(g, grp(part, g))

        def op_P(gk):
            gqs = [gq for gq in range(NG) if visible(gq, gk)]
            vals = jnp.concatenate([vt[gk, c] for c in range(4)], axis=1)
            part = dot_PV(jnp.concatenate(
                [ps[gk, 8 * gq:8 * gq + 8, :] if 'p' in STORE else probs[gq, gk] for gq in gqs], axis=0), vals)
            for i, gq in enumerate(gqs):
                accumulate(gq, grp(part, i))

        def op_M(i):
            if mix is not None:
                mix(i)

        table = dict(U=(op_U, NP), T=(op_T, NP), V=(op_V, NP), C=(op_C, NG), D=(op_D, NG), X=(op_X, NG),
                     A=(op_A, 8), P=(op_P, NG), M=(op_M, 2))
        for tok in ORDER.split():
            fn, n = table[tok[0]]
            for i in ([int(ch) for ch in tok[1:]] if len(tok) > 1 else range(n)):
                fn(i)
        o = jnp.concatenate(rows, axis=0)
        ob = o[:, DA:]
        o = jnp.concatenate([o[:, :DA], ob + pltpu.roll(ob, 64, 1)], axis=1)
        return o[:M], o[M:]

    def finish_block(b):
        oT = jnp.concatenate([onat[:, 128 * c:128 * (c + 1)].T for c in range(4)], axis=0)
        hb = xT[b].astype(F32) + oT[0:D]
        hT[b] = hb
        hnT[...] = _ln_rows(_ln_rows(hb))

    def mix_rows(b, r, i):
        rows = pl.ds(112 * r, 112)
        cols = pl.ds(F // 2 * i, F // 2)
        u[rows, cols] += dot_MX(hnT[rows, :], w1[pl.ds(_aligned(b, 128), 128), cols])

    def block(b, mem, first):
        if not first:
            finish_block(b - 1)
        for r in range(STEPS):
            mem, o = step(mem, 4 * b + r, None if first else (lambda i: mix_rows(b - 1, r, i)))
            onat[SEG * r:SEG * (r + 1), :] = o
            if r == 0:
                prep_x(1 if first else jnp.minimum(b + 1, NB - 1))
        return mem

    m0 = mem_ref[0].astype(F32)
    mem = jnp.concatenate([m0, m0[:, DA:D]], axis=1)

    def prefetch(b):
        @pl.when(b + 1 < NB)
        def _():
            x_copy(b + 1).wait()

        @pl.when(b + 2 < NB)
        def _():
            x_copy(b + 2).start()
        w1_copy(b).start()
        w2_copy(b).start()

    if not ONLY_LOOP:
        prefetch(0)
        with _scope("block0"):
            mem = block(0, mem, True)

    def loop_body(b, m):
        if not ONLY_LOOP:
            prefetch(b)
            w1_copy(b - 1).wait()
        with _scope("block"):
            return block(b, m, False)

    mem = lax.fori_loop(1, NB, loop_body, mem)
    if ONLY_LOOP:
        ostage[0:16, 0:512] = jnp.concatenate([mem, mem], axis=0).astype(BF16)
        cp = pltpu.make_async_copy(ostage, out_hbm, osem.at[0])
        cp.start()
        cp.wait()
        return

    w1_copy(NB - 1).wait()
    for b in range(NB):
        w2_copy(b).wait()
    with _scope("tail_u"):
        finish_block(NB - 1)
        for r in range(4):
            for i in range(2):
                mix_rows(NB - 1, r, i)
    b2 = b2_ref[...].astype(F32).reshape(1, S)
    out_copies = []
    for r in range(4):
        rows = pl.ds(112 * r, 112)
        with _scope("tail_y"):
            g = jax.nn.gelu(u[rows, :], approximate=True)
            y = dot_Y(g, w2[...]) + b2
            res = jnp.concatenate([hT[b, rows, :] for b in range(NB)], axis=1)
            ostage[rows, :] = (res + y).astype(BF16)
        cp = pltpu.make_async_copy(ostage.at[rows, :], out_hbm.at[rows, :], osem.at[r])
        cp.start()
        out_copies.append(cp)
    with _scope("out_wait"):
        for cp in out_copies:
            cp.wait()


@jax.jit
def pallas_sequential_preLN__memory_aug_recurrent_mem_tr__mixer_token_mlp__prompt_kernel(A_x, A_mem0, A_Wq, A_Wk, A_Wv, A_Wo, A_seg_len, B_x, B_w1, B_b1, B_w2, B_b2):
    del A_seg_len, B_x
    hbm = pl.BlockSpec(memory_space=pl.ANY)
    vmem = pl.BlockSpec(memory_space=pltpu.VMEM)
    out = pl.pallas_call(
        _kernel,
        out_shape=jax.ShapeDtypeStruct((D, S), BF16),
        in_specs=[hbm, vmem, hbm, hbm, hbm, hbm, hbm, vmem, hbm, vmem],
        out_specs=hbm,
        scratch_shapes=[
            pltpu.VMEM((3, NP, D, E), U32),
            pltpu.VMEM((H, D, E), BF16),
            pltpu.VMEM((NB, D, 128), BF16),
            pltpu.VMEM((NP, DA // 2, PW), U32),
            pltpu.VMEM((NP, D // 2, 128), U32),
            pltpu.VMEM((NP, DA // 2, PW), U32),
            pltpu.VMEM((8, 64, DP), U32),
            pltpu.VMEM((S, DP), F32),
            pltpu.VMEM((S, F), BF16),
            pltpu.VMEM((F, S), BF16),
            pltpu.VMEM((NG, 4, 128, 128), BF16),
            pltpu.VMEM((NG, 128, 128), BF16),
            pltpu.VMEM((NG, 4, 128, 128), BF16),
            pltpu.VMEM((NG, L, 128), F32),
            pltpu.VMEM((NG, L, 128), F32),
            pltpu.VMEM((8, L, 128), F32),
            pltpu.VMEM((128, DP), F32),
            pltpu.VMEM((NB, D, 128), F32),
            pltpu.VMEM((D, 128), F32),
            pltpu.VMEM((D, F), F32),
            pltpu.VMEM((D, S), BF16),
            pltpu.SemaphoreType.DMA((4, NP)),
            pltpu.SemaphoreType.DMA((NB,)),
            pltpu.SemaphoreType.DMA((2, NB)),
            pltpu.SemaphoreType.DMA((4,)),
        ],
        compiler_params=pltpu.CompilerParams(vmem_limit_bytes=100 * 2 ** 20, flags=FLAGS),
        name="rmt_mixer",
    )(
        jnp.transpose(A_x, (0, 2, 1)).reshape(D, S),
        A_mem0, A_Wq, A_Wk, A_Wv,
        jnp.transpose(A_Wo, (0, 2, 1)),
        B_w1, B_b1, B_w2, B_b2,
    )
    return jnp.transpose(out.reshape(1, D, S), (0, 2, 1))
```

```python
import functools

import jax
import jax.experimental.pallas as pl
import jax.experimental.pallas.tpu as pltpu
import jax.numpy as jnp
import numpy as np
from jax import lax

F32 = jnp.float32
BF16 = jnp.bfloat16
U32 = jnp.uint32

S, D, H, E, M, SEG, F = 2048, 448, 16, 256, 8, 32, 1792
DA = 384
DB = D - DA
DP = DA + 2 * DB
L = M + SEG
NG = L // 8
NB = S // 128
NI = NB // 2
NP = H // 2
PW = 2 * D
DH, FH, SH = D // 2, F // 2, S // 2
FT = FH // 128
YC = 2
YW = SH // YC
LAST = 4
EPS = 1e-5
SCALE = E ** -0.5
LOG2E = 1.4426950408889634
GELU_C = 0.7978845608028654

LEFT = ((0, 3, 1), (2, 3, 1), (0, None, 0), (3, None, 0), (0, 1, 1), (2, 0, -1), (1, 3, -1))
RIGHT = ((0, 3, 1), (0, None, 0), (1, 3, -1), (2, 0, -1), (3, None, 0), (0, 1, 1), (2, 3, 1))
MERGE = (((0, 1), (3, 1), (4, -1), (6, 1)), ((2, 1), (4, 1)),
         ((1, 1), (3, 1)), ((0, 1), (1, -1), (2, 1), (5, 1)))
MIX_UNITS = tuple((m, n) for m in (2, 5, 0, 1, 3, 4, 6) for n in range(FT))

STEP_ORDER = ("U1 U3 U2 U4 U0 U5 U7 U6 T0 T1 C3 T2 C0 T3 C2 T4 C1 C4 T5 T6 T7 "
              "V0 D1 V1 D0 V2 D2 X1 V3 X0 D3 X2 V4 D4 X3 V5 X4 V6 M0 V7 "
              "A0 A3 A1 A4 A2 A7 A5 P2 P0 P3 A6 P1 P4 M1")
TAIL_HEAD = "N0 M0 M1 M2 g3 y3 M3 g2 y1 M4 g1 y6 M5 g0 y4 M6 y0 y2 y5 G3 Y3 G2 Y1 G1 G0 Y6 E2"
TAIL_BODY = "Y4 Y0 E0 Y2 E1 Z5"


def _dot(a, b):
    return jnp.dot(a, b, preferred_element_type=F32)


def _dot_nt(a, b):
    return lax.dot_general(a, b, (((1,), (1,)), ((), ())), preferred_element_type=F32)


def _layernorm(x):
    c = x - jnp.mean(x, axis=0, keepdims=True)
    return c * lax.rsqrt(jnp.mean(c * c, axis=0, keepdims=True) + EPS)


def _lanes(rows):
    return lax.broadcasted_iota(jnp.int32, (rows, 128), 1)


def _sublanes():
    return lax.broadcasted_iota(jnp.int32, (8, 128), 0)


def _swap8(v):
    v = pltpu.roll(v, 0, 1, stride=1, stride_axis=0)
    v = jnp.take_along_axis(v, (_sublanes() + _lanes(8) + 1) & 7, axis=0)
    v = pltpu.roll(v, 121, 1, stride=1, stride_axis=0)
    return jnp.take_along_axis(v, 7 - _sublanes(), axis=0)


def _transpose(x):
    return jnp.concatenate([x[:, c:c + 128].T for c in range(0, x.shape[1], 128)], axis=0)


def _words(x):
    return pltpu.bitcast(x.astype(BF16), U32)


def _group(x, g):
    return x[8 * g:8 * (g + 1)]


def _visible(gq, gk):
    return gq == 0 or gk <= gq


def _combine(load, spec):
    a, b, sign = spec
    if b is None:
        return load(a)
    x, y = load(a).astype(F32), load(b).astype(F32)
    return x + y if sign > 0 else x - y


def _merge(load, quadrant):
    (first, _), *rest = MERGE[quadrant]
    total = load(first)
    for m, sign in rest:
        total = total + load(m) if sign > 0 else total - load(m)
    return total


def _aligned(i, n):
    return i * n if isinstance(i, int) else pl.multiple_of(i * n, n)


def _kernel(xT_hbm, mem_hbm, wq_hbm, wk_hbm, wv_hbm, woT_hbm, w1_hbm, b1_hbm, w2_hbm, b2_hbm,
            out_hbm,
            wraw, woT, xT, wp, wu, wz, xn, w1, w2, tt, ut, vt, zb, onat, hT, hn, uacc, act, yacc,
            ostage, memc, bias2, mem0, b1_ref, b2_ref, zero,
            wsem, xsem, msem, osem):
    def raw_copy(n, w, p):
        return pltpu.make_async_copy(w.bitcast(U32).at[:, p, :], wraw.at[n, p], wsem.at[n, p])

    def qk_copies(p):
        return [raw_copy(0, wq_hbm, p), raw_copy(1, wk_hbm, p)]

    def vo_copies(p):
        heads = pl.ds(2 * p, 2)
        return [raw_copy(2, wv_hbm, p),
                pltpu.make_async_copy(woT_hbm.at[heads], woT.at[heads], wsem.at[3, p])]

    def x_copy(k):
        cols = (pl.ds(0, 128), pl.ds(128, 256), pl.ds(384, S - 384))[k]
        return pltpu.make_async_copy(xT_hbm.at[:, cols], xT.at[:, cols], xsem.at[k])

    def small_copies():
        pairs = ((mem_hbm, mem0), (b1_hbm, b1_ref), (b2_hbm, b2_ref))
        return [pltpu.make_async_copy(src, dst, xsem.at[3 + j]) for j, (src, dst) in enumerate(pairs)]

    def w1_copy():
        return pltpu.make_async_copy(w1_hbm, w1.at[pl.ds(256, S)], msem.at[0])

    def w2_copies():
        return [pltpu.make_async_copy(w2_hbm.at[:, pl.ds(YW * j, YW)], w2.at[j], msem.at[1 + j])
                for j in range(2 * YC)]

    def out_copy(q, c, part=0):
        rows, j = pl.ds(DH * (q // 2), DH), YC * (q % 2) + c
        w = YW // (LAST if q == 3 else 1)
        return pltpu.make_async_copy(ostage.at[j, rows, pl.ds(w * part, w)],
                                     out_hbm.at[rows, pl.ds(_aligned(j * (YW // w) + part, w), w)],
                                     osem.at[q + part, c])

    def head_pair(n, p):
        packed = wraw[n, p]
        even = pltpu.bitcast(packed << 16, F32)
        odd = pltpu.bitcast(packed & np.uint32(0xFFFF0000), F32)
        return even, odd

    def pair_products(l0, l1, r0, r1):
        tail = jnp.concatenate([l0[DA:], l1[DA:]], axis=0)
        rest = [_dot_nt(r[DA:], jnp.concatenate([l[:DA], tail], axis=0).astype(BF16))
                for l, r in ((l0, r0), (l1, r1))]
        main = [_dot_nt(jnp.concatenate([l[DA:], l[:DA]], axis=0), r[:DA].astype(BF16))
                for l, r in ((l0, r0), (l1, r1))]
        return [(m[DB:], m[:DB]) for m in main], rest

    def absorb_qk(p):
        ((m0, t0), (m1, t1)), (r0, r1) = pair_products(*head_pair(0, p), *head_pair(1, p))
        shared = _transpose(jnp.concatenate([r0[:, :DA], r1[:, :DA]], axis=0))
        keyside = jnp.concatenate([_transpose(jnp.concatenate([t0, t1], axis=0)),
                                   jnp.where(_lanes(DB) < DB, r0[:, DA:], r1[:, DA:])], axis=0)
        wu[p] = _words(keyside)
        wp[p] = _words(jnp.concatenate([m0, m1, shared], axis=1))

    def absorb_vo(p):
        ((m0, t0), (m1, t1)), (r0, r1) = pair_products(*head_pair(2, p), woT[2 * p], woT[2 * p + 1])
        shared = _transpose(jnp.concatenate([r0, r1], axis=0))
        low = _lanes(DB) < DB
        z0 = jnp.concatenate([t0, jnp.where(low, shared[DA:D], 0.0)], axis=1)
        z1 = jnp.concatenate([t1, jnp.where(low, 0.0, shared[D:])], axis=1)
        for dg in range(DB // 8):
            wz[dg, pl.ds(_aligned(p, 8), 8), :] = _words(
                jnp.concatenate([_group(z0, dg), _group(z1, dg)], axis=0))
        wp[NP + p] = _words(jnp.concatenate([m0, m1, shared[:DA]], axis=1))

    def absorb_all(copies, absorb):
        def body(p, carry):
            for c in copies(p):
                c.wait()
            absorb(p)
            return carry
        lax.fori_loop(0, NP, body, 0)

    def normalize_x(b):
        n = _layernorm(xT[:, pl.ds(_aligned(b, 128), 128)].astype(F32))
        n = jnp.concatenate([n, n[DA:]], axis=0)
        for c in range(DP // 128):
            xn[pl.ds(_aligned(b, 128), 128), 128 * c:128 * (c + 1)] = n[128 * c:128 * (c + 1)].T

    def put_pair(dst, even, odd, p):
        for g in range(NG):
            dst(g)[pl.ds(16 * p, 16), :] = jnp.concatenate(
                [_group(even, g), _group(odd, g)], axis=0).astype(BF16)

    def project(h, first, dst, p):
        t = _dot(h[:, :DA], pltpu.bitcast(wp[first + p], BF16))
        for c in range(3):
            put_pair(lambda g: dst.at[g, c],
                     t[:, 128 * c:128 * (c + 1)], t[:, DA + 128 * c:DA + 128 * (c + 1)], p)
        shared, low = t[:, 2 * DA:], _lanes(L) < DB
        put_pair(lambda g: dst.at[g, 3], jnp.where(low, shared, 0.0), jnp.where(low, 0.0, shared), p)

    def step(mem, seg, mix):
        h = jnp.concatenate([mem, xn[pl.ds(_aligned(seg, SEG), SEG), :]], axis=0)
        hb = h[:, DA:]
        hbT = jnp.concatenate([hb, jnp.zeros((128 - L, 128), F32)], axis=0).T[:DB]
        cross, direct, probs = {}, {}, {}
        rows = [None] * NG

        def accumulate(g, v):
            rows[g] = v if rows[g] is None else rows[g] + v

        def key_side(p):
            t = _dot(h[:, :D], pltpu.bitcast(wu[p], BF16))
            low = _lanes(L) < DB
            put_pair(lambda g: ut.at[g], jnp.where(low, t, 0.0), jnp.where(low, 0.0, t), p)

        def cross_scores(gk):
            gqs = [gq for gq in range(NG) if _visible(gq, gk)]
            s = _dot_nt(jnp.concatenate([_group(hb, gq) for gq in gqs], axis=0), ut[gk])
            for i, gq in enumerate(gqs):
                cross[gq, gk] = _swap8(_group(s, i))

        def direct_scores(gq):
            n = sum(_visible(gq, gk) for gk in range(NG))
            queries = jnp.concatenate([tt[gq, c] for c in range(4)], axis=1)
            direct[gq] = _dot_nt(h[:8 * n], queries)

        def softmax(gq):
            n = direct[gq].shape[0] // 8
            parts = []
            for gk in range(n):
                s = _group(direct[gq], gk) + cross[gq, gk]
                if gq > 0 and gk == gq:
                    s = jnp.where(_sublanes() <= (_lanes(8) & 7), s, -1e9 / SCALE)
                parts.append(s)
            s = jnp.concatenate(parts, axis=0)
            e = jnp.exp2((s - jnp.max(s, axis=0, keepdims=True)) * (SCALE * LOG2E))
            pt = e * (1.0 / jnp.sum(e, axis=0, keepdims=True))
            for gk in range(n):
                probs[gq, gk] = _swap8(_group(pt, gk))
            if n % 2:
                pt = jnp.concatenate([pt, jnp.zeros((8, 128), F32)], axis=0)
            zT = _dot(hbT[:, :pt.shape[0]], pt.astype(BF16))
            for dg in range(DB // 8):
                zb[dg, 8 * gq:8 * gq + 8, :] = _swap8(_group(zT, dg))

        def late_values(dg):
            part = _dot(zb[dg + zero[0] if dg == 0 else dg], pltpu.bitcast(wz[dg], BF16))
            for g in range(NG):
                accumulate(g, _group(part, g))

        def early_values(gk):
            gqs = [gq for gq in range(NG) if _visible(gq, gk)]
            values = jnp.concatenate([vt[gk, c] for c in range(4)], axis=1)
            part = _dot(jnp.concatenate([probs[gq, gk] for gq in gqs], axis=0), values)
            for i, gq in enumerate(gqs):
                accumulate(gq, _group(part, i))

        pieces = dict(U=key_side, T=functools.partial(project, h, 0, tt),
                      V=functools.partial(project, h, NP, vt), C=cross_scores, D=direct_scores,
                      X=softmax, A=late_values, P=early_values, M=mix)
        for name, index in STEP_ORDER.split():
            pieces[name](int(index))
        o = jnp.concatenate(rows, axis=0)
        ob = o[:, DA:]
        o = jnp.concatenate([o[:, :DA], ob + pltpu.roll(ob, DB, 1)], axis=1)
        return o[:M], o[M:]

    def finish_block(b, half):
        oT = _transpose(onat[128 * half:128 * (half + 1), :])
        cols = pl.ds(_aligned(b if isinstance(b, int) else jnp.maximum(b, 0), 128), 128)
        hT[b + 1] = xT[:, cols].astype(F32) + oT[:D]

    def normalize_block(b):
        n = _layernorm(_layernorm(hT[b + 1]))
        hn[2 * b + 4] = n[:DH]
        hn[2 * b + 5] = n[DH:]

    def mix_unit(i, m, n, parts=1):
        def load(q):
            return w1[pl.ds(_aligned(2 * i + 2 + q // 2, 128), 128), pl.ds(FH * (q % 2) + 128 * n, 128)]
        cols = pl.ds(128 * n, 128)
        w = _combine(load, RIGHT[m]).astype(BF16)
        for k in range(parts):
            rows = pl.ds(DH // parts * k, DH // parts)
            x = _combine(lambda q: hn[4 * i + 4 + 2 * (q % 2) + q // 2, rows, :], LEFT[m])
            total = uacc[m, rows, cols] + _dot(x, w)
            uacc[m, rows, cols] = total if isinstance(i, int) else jnp.where(i >= 0, total, 0.0)

    def iteration(i):
        finish_block(2 * i - 1, 1)
        mem = memc[...]
        for r in range(8):
            def mix(part, r=r):
                lo, hi = (6 * r, 6 * r + 2) if part == 0 else (6 * r + 2, 6 * r + 6 + (r == 7))
                for m, n in MIX_UNITS[lo:hi]:
                    mix_unit(i - 1, m, n, 2 + 2 * part)
            mem, o = step(mem, 8 * i + r, mix)
            onat[SEG * r:SEG * (r + 1), :] = o
            if r == 0:
                normalize_block(2 * i - 1)
            if r == 2:
                normalize_x(2 * i + 1)
            if r == 3:
                finish_block(2 * i, 0)
                normalize_block(2 * i)
            if r == 6:
                normalize_x(2 * i + 2)
        memc[...] = mem

    def activate(q, lo, hi):
        cols = pl.ds(128 * lo, 128 * (hi - lo))
        first = FH * (q % 2) + 128 * lo
        b1 = b1_ref[...].astype(F32).reshape(1, F)[:, first:first + 128 * (hi - lo)]
        u = _merge(lambda m: uacc[m, :, cols], q) + b1
        t = jnp.tanh(u * (GELU_C + (GELU_C * 0.044715) * (u * u)))
        half = 0.5 * u
        act[q, :, cols] = half + half * t

    def project_out(m, c, lo, hi, cols=slice(None)):
        def load(q):
            return w2[YC * (q % 2) + c, pl.ds(FH * (q // 2) + 128 * lo, 128 * (hi - lo)), cols]
        x = _combine(lambda q: act[q, :, pl.ds(128 * lo, 128 * (hi - lo))], LEFT[m])
        y = _dot(x, _combine(load, RIGHT[m]).astype(BF16))
        yacc[m, c, :, cols] = y if lo == 0 else yacc[m, c, :, cols] + y

    def emit(q, c, part=0):
        rows, j = pl.ds(DH * (q // 2), DH), YC * (q % 2) + c
        w = YW // (LAST if q == 3 else 1)
        cols = pl.ds(w * part, w)
        first = j * (YW // 128) + part * (w // 128) + 1
        res = jnp.concatenate([hT[first + k, rows, :] for k in range(w // 128)], axis=1)
        y = _merge(lambda m: yacc[m, c, :, cols], q)
        ostage[j, rows, cols] = (res + y + bias2[j, :, cols]).astype(BF16)
        out_copy(q, c, part).start()

    def run_tail(order, chunks):
        for name, index in order.split():
            i = int(index)
            lo, hi = (0, 1) if name.islower() else (1, FT)
            if name == "N":
                for m, n in MIX_UNITS[:2 * FT]:
                    mix_unit(NI - 1, m, n)
            elif name == "M":
                for m in (0, 1, 3, 4, 6):
                    mix_unit(NI - 1, m, i)
            elif name in "gG":
                activate(i, lo, hi)
            for c in chunks:
                if name in "yY":
                    project_out(i, c, lo, hi)
                elif name == "E":
                    emit(i, c)
                elif name == "Z":
                    for part in range(LAST):
                        project_out(i, c, lo, hi, pl.ds(YW // LAST * part, YW // LAST))
                        emit(3, c, part)

    def tail():
        for c in w2_copies():
            c.wait()
        finish_block(NB - 1, 1)
        normalize_block(NB - 1)
        run_tail(TAIL_HEAD, range(YC))

        def chunk(c, carry):
            run_tail(TAIL_BODY, [c])
            return carry
        lax.fori_loop(0, YC, chunk, 0)
        for c in range(YC):
            for q in range(3):
                out_copy(q, c).wait()
            for part in range(LAST):
                out_copy(3, c, part).wait()

    zero[0] = 0
    x_copy(0).start()
    for copies in (qk_copies, vo_copies):
        def start(p, carry, copies=copies):
            for c in copies(p):
                c.start()
            return carry
        lax.fori_loop(0, NP, start, 0)
    x_copy(1).start()
    for c in small_copies():
        c.start()
    x_copy(0).wait()
    normalize_x(0)
    absorb_all(qk_copies, absorb_qk)
    absorb_all(vo_copies, absorb_vo)
    x_copy(1).wait()
    for c in small_copies():
        c.wait()
    x_copy(2).start()
    w1_copy().start()
    for c in w2_copies():
        c.start()

    m0 = mem0[0].astype(F32)
    memc[...] = jnp.concatenate([m0, m0[:, DA:]], axis=1)
    b2 = b2_ref[...].astype(F32).reshape(1, S)
    for j in range(2 * YC):
        bias2[j] = b2[:, YW * j:YW * (j + 1)]

    def body(i, carry):
        @pl.when(i < NI)
        def _():
            @pl.when(i == 1)
            def _():
                x_copy(2).wait()
                w1_copy().wait()
            iteration(i)

        pl.when(i == NI)(tail)
        return carry

    lax.fori_loop(0, NI + 1, body, 0)


@functools.partial(jax.jit, static_argnames=("A_seg_len",))
def pallas_sequential_preLN__memory_aug_recurrent_mem_tr__mixer_token_mlp__prompt_kernel(
    A_x: jax.Array,
    A_mem0: jax.Array,
    A_Wq: jax.Array,
    A_Wk: jax.Array,
    A_Wv: jax.Array,
    A_Wo: jax.Array,
    A_seg_len: int,
    B_x: jax.Array,
    B_w1: jax.Array,
    B_b1: jax.Array,
    B_w2: jax.Array,
    B_b2: jax.Array,
):
    del B_x
    assert A_seg_len == SEG and A_x.shape == (1, S, D) and A_mem0.shape == (1, M, D)
    assert A_Wq.shape == (D, H, E) and A_Wo.shape == (H, E, D) and B_w1.shape == (S, F)
    hbm = pl.BlockSpec(memory_space=pl.ANY)
    out = pl.pallas_call(
        _kernel,
        out_shape=jax.ShapeDtypeStruct((D, S), BF16),
        in_specs=[hbm] * 10,
        out_specs=hbm,
        scratch_shapes=[
            pltpu.VMEM((3, NP, D, E), U32),
            pltpu.VMEM((H, D, E), BF16),
            pltpu.VMEM((D, S + 128), BF16),
            pltpu.VMEM((2 * NP, DA // 2, PW), U32),
            pltpu.VMEM((NP, D // 2, 128), U32),
            pltpu.VMEM((DB // 8, 64, DP), U32),
            pltpu.VMEM((S + 128, DP), F32),
            pltpu.VMEM((S + 256, F), BF16),
            pltpu.VMEM((2 * YC, F, YW), BF16),
            pltpu.VMEM((NG, 4, 128, 128), BF16),
            pltpu.VMEM((NG, 128, 128), BF16),
            pltpu.VMEM((NG, 4, 128, 128), BF16),
            pltpu.VMEM((DB // 8, L, 128), F32),
            pltpu.VMEM((256, DP), F32),
            pltpu.VMEM((NB + 1, D, 128), F32),
            pltpu.VMEM((2 * NB + 4, DH, 128), F32),
            pltpu.VMEM((7, DH, FH), F32),
            pltpu.VMEM((4, DH, FH), F32),
            pltpu.VMEM((7, YC, DH, YW), F32),
            pltpu.VMEM((2 * YC, D, YW), BF16),
            pltpu.VMEM((M, DP), F32),
            pltpu.VMEM((2 * YC, 1, YW), F32),
            pltpu.VMEM((1, M, D), BF16),
            pltpu.VMEM((F,), BF16),
            pltpu.VMEM((S,), BF16),
            pltpu.SMEM((1,), jnp.int32),
            pltpu.SemaphoreType.DMA((4, NP)),
            pltpu.SemaphoreType.DMA((6,)),
            pltpu.SemaphoreType.DMA((1 + 2 * YC,)),
            pltpu.SemaphoreType.DMA((3 + LAST, YC)),
        ],
        compiler_params=pltpu.CompilerParams(vmem_limit_bytes=110 * 2 ** 20),
        name="rmt_mixer",
    )(
        jnp.transpose(A_x, (0, 2, 1)).reshape(D, S),
        A_mem0, A_Wq, A_Wk, A_Wv,
        jnp.transpose(A_Wo, (0, 2, 1)),
        B_w1, B_b1, B_w2, B_b2,
    )
    return jnp.transpose(out.reshape(1, D, S), (0, 2, 1))
```

```python
import functools

import jax
import jax.experimental.pallas as pl
import jax.experimental.pallas.tpu as pltpu
import jax.numpy as jnp
import numpy as np
from jax import lax

F32 = jnp.float32
BF16 = jnp.bfloat16
U32 = jnp.uint32

S, D, H, E, M, SEG, F = 2048, 448, 16, 256, 8, 32, 1792
DA = 384
DB = D - DA
DP = DA + 2 * DB
L = M + SEG
NG = L // 8
NB = S // 128
NI = NB // 2
NP = H // 2
DH, FH, SH = D // 2, F // 2, S // 2
FT = FH // 128
YC = 2
YW = SH // YC
LAST = 4
EPS = 1e-5
SCALE = E ** -0.5
LOG2E = 1.4426950408889634
GELU_C = 0.7978845608028654

LEFT = ((0, 3, 1), (2, 3, 1), (0, None, 0), (3, None, 0), (0, 1, 1), (2, 0, -1), (1, 3, -1))
RIGHT = ((0, 3, 1), (0, None, 0), (1, 3, -1), (2, 0, -1), (3, None, 0), (0, 1, 1), (2, 3, 1))
MERGE = (((0, 1), (3, 1), (4, -1), (6, 1)), ((2, 1), (4, 1)),
         ((1, 1), (3, 1)), ((0, 1), (1, -1), (2, 1), (5, 1)))
MIX_UNITS = tuple((m, n) for m in (2, 5, 0, 1, 3, 4, 6) for n in range(FT))

A_, B_, C_, D_, E_, F_, G_ = range(7)
M1, M2, M12 = (1, 0), (0, 1), (1, 1)
PASSES = (
    ((A_, M1, (1, -1), 0, 24), (E_, M12, (-1, 1), 8, 32), (F_, M1, (0, 1), 0, 32), (G_, M2, (1, 0), 0, 32)),
    ((A_, M12, (0, 1), 24, 48), (C_, M1, (0, 1), 16, 40), (B_, M12, (1, -1), 0, 32), (D_, M2, (1, 0), 0, 32)),
    ((B_, M12, (1, 0), 32, 56), (C_, M1, (0, 1), 40, 64), (D_, M2, (1, 0), 32, 64), (E_, M12, (0, 1), 32, 64)),
    ((A_, M2, (-1, 1), 48, 72), (B_, M12, (1, -1), 56, 80), (F_, M1, (0, 1), 32, 64), (G_, M2, (1, 0), 32, 64)),
    ((A_, M12, (1, 0), 72, 96), (E_, M12, (-1, 1), 64, 88), (C_, M1, (0, 1), 64, 96), (D_, M2, (1, 0), 64, 96)),
    ((B_, M1, (1, -1), 80, 104), (E_, M2, (-1, 1), 88, 112), (F_, M1, (0, 1), 64, 96), (G_, M2, (1, 0), 64, 96)),
    ((B_, M12, (1, -1), 104, 128), (C_, M1, (0, 1), 96, 120), (A_, M12, (0, 1), 96, 128), (D_, M2, (1, 0), 96, 128)),
    ((C_, M1, (-1, 1), 120, 144), (E_, M12, (-1, 1), 112, 136), (F_, M1, (1, 0), 96, 128), (G_, M2, (1, 0), 96, 128)),
)
RING = (128, 128, 128, 64, 128, 64, 64)
BASE = (0, 128, 256, 384, 448, 576, 640)
SAVED = BASE[-1] + RING[-1]
FIRST_ROWS = (32, 32, 48, 32, 40, 32, 32)

STEP_ORDER = (
    "U0 U1 U2 U3 T0 T1 C1 T2 C0 T3 C2 T4 C3 C4 T5 T6 T7 "
    "V0 D1 M0 V1 D0 V2 D2 X1 Z1 V3 X0 Z0 D3 X2 Z2 V4 D4 X3 Z3 V5 X4 Z4 V6 M1 V7 "
    "A0 A2 A1 P2 P3 A3 P0 P1 P4 M2",
    "U0 U1 U2 U3 T0 T1 C3 T2 C0 T3 C2 T4 C1 C4 T5 T6 T7 "
    "V0 D1 M0 V1 D0 V2 D2 X1 Z1 V3 X0 Z0 D3 X2 Z2 V4 D4 X3 Z3 V5 X4 Z4 V6 M1 V7 "
    "A0 A2 A1 P2 P0 P3 A3 P1 P4 M2",
    "U0 U1 U2 U3 T0 T1 C3 T2 C0 T3 C2 T4 C1 C4 T5 T6 T7 "
    "V0 D1 M0 V1 D0 V2 D2 X1 Z1 V3 X0 Z0 D3 X2 Z2 V4 D4 X3 Z3 V5 X4 Z4 V6 M1 V7 "
    "A0 A2 A1 P2 P0 P3 A3 P4 P1 M2",
    "U0 U1 U2 U3 T0 T1 C4 T2 C0 T3 C2 T4 C1 C3 T5 T6 T7 "
    "V0 D1 M0 V1 D0 V2 D2 X1 Z1 V3 X0 Z0 D3 X2 Z2 V4 D4 X3 Z3 V5 X4 Z4 V6 M1 V7 "
    "A0 A2 A1 P2 P0 P3 A3 P1 P4 M2",
    "U0 U1 U2 U3 T0 T1 C3 T2 C0 T3 C2 T4 C1 C4 T5 T6 T7 "
    "V0 D1 M0 V1 D0 V2 D2 X1 Z1 V3 X0 Z0 X2 D3 X3 Z2 V4 D4 Z3 V5 X4 Z4 V6 M1 V7 "
    "A0 A2 A1 P2 P0 P3 A3 P1 P4 M2",
    "U0 U1 U2 U3 T0 T1 C3 T2 C0 T3 C2 T4 C1 C4 T5 T6 T7 "
    "V0 D1 M0 V1 D0 V2 D2 X1 Z1 V3 X0 Z0 D3 X2 Z2 V4 D4 X3 Z3 V5 X4 Z4 V6 M1 V7 "
    "A0 A2 A1 P2 P0 P3 A3 P1 P4 M2",
    "U0 U1 U2 U3 T0 T1 C3 T2 C0 T3 C2 T4 C1 C4 T5 T6 T7 "
    "V0 D1 M0 V1 D0 V2 D2 X1 Z1 V3 X0 Z0 D3 X2 Z2 V4 D4 X3 Z3 V5 X4 Z4 V6 M1 V7 "
    "A0 A2 A1 P2 P0 P3 A3 P1 P4 M2",
    "U0 U1 U2 U3 T0 T1 C3 T2 C0 T3 C2 T4 C4 C1 T5 T6 T7 "
    "V0 D1 M0 V1 D0 V2 D2 X1 X2 V3 Z1 X0 Z0 D3 Z2 V4 D4 X3 Z3 V5 X4 Z4 V6 M1 V7 "
    "A0 A2 A1 P2 P0 P3 A3 P1 P4 M2",
)
PROJECT_ORDER = (("a01b2H3", "01Hab23"), ("0a1b2H3", "012RH3"), ("a1b20H3", "10b2Ha3"),
                 ("0a1b2H3", "02a1bH3"), ("0a1b2H3", "0a1b2H3"), ("0a1b2H3", "0a1b2H3"),
                 ("0a1b2H3", "0a1b2H3"), ("0a1b2H3", "0a1b32H"))
MIX_SPLIT = (((1, 1, 4), (2, 4, 4)), ((1, 1, 4), (2, 4, 4)), ((1, 1, 4), (2, 4, 4)),
             ((1, 1, 4), (2, 4, 4)), ((1, 1, 4), (2, 4, 4)), ((1, 1, 4), (2, 4, 4)),
             ((1, 1, 4), (2, 4, 4)), ((1, 1, 4), (2, 4, 4)))
CHORES = ("N", "n", "FL", "", "", "", "f", "l")
PINS = ((0, 1), (1, 1), (2, 1), (6, 1), (7, 1))
TAIL_HEAD = "N0 M0 M1 M2 g3 y3 M3 g2 y1 M4 g1 y6 M5 g0 y4 M6 y0 y2 y5 G3 Y3 G2 Y1 G1 G0 Y6 E2"
TAIL_BODY = "Y4 Y0 E0 Y2 E1 Z5"


def _dot(a, b):
    return jnp.dot(a, b, preferred_element_type=F32)


def _dot_nt(a, b):
    return lax.dot_general(a, b, (((1,), (1,)), ((), ())), preferred_element_type=F32)


def _layernorm(x):
    c = x - jnp.mean(x, axis=0, keepdims=True)
    return c * lax.rsqrt(jnp.mean(c * c, axis=0, keepdims=True) + EPS)


def _double_layernorm(x):
    c = x - jnp.mean(x, axis=0, keepdims=True)
    var = jnp.mean(c * c, axis=0, keepdims=True)
    rest = jnp.mean(c, axis=0, keepdims=True)
    first = lax.rsqrt(var + EPS)
    second = lax.rsqrt((var - rest * rest) * first * first + EPS)
    return (c - rest) * (first * second)


def _lanes(rows):
    return lax.broadcasted_iota(jnp.int32, (rows, 128), 1)


def _sublanes():
    return lax.broadcasted_iota(jnp.int32, (8, 128), 0)


def _swap8(v):
    v = pltpu.roll(v, 0, 1, stride=1, stride_axis=0)
    v = jnp.take_along_axis(v, (_sublanes() + _lanes(8) + 1) & 7, axis=0)
    v = pltpu.roll(v, 121, 1, stride=1, stride_axis=0)
    return jnp.take_along_axis(v, 7 - _sublanes(), axis=0)


def _transpose(x):
    return jnp.concatenate([x[:, c:c + 128].T for c in range(0, x.shape[1], 128)], axis=0)


def _words(x):
    return pltpu.bitcast(x.astype(BF16), U32)


def _group(x, g):
    return x[8 * g:8 * (g + 1)]


def _visible(gq, gk):
    return gq == 0 or gk <= gq


def _combine(load, spec):
    a, b, sign = spec
    if b is None:
        return load(a)
    x, y = load(a).astype(F32), load(b).astype(F32)
    return x + y if sign > 0 else x - y


def _merge(load, terms):
    (first, _), *rest = terms
    total = load(first)
    for m, sign in rest:
        total = total + load(m) if sign > 0 else total - load(m)
    return total


def _aligned(i, n):
    return i * n if isinstance(i, int) else pl.multiple_of(i * n, n)


def _kernel(xT_hbm, mem_hbm, wq_hbm, wk_hbm, wv_hbm, woT_hbm, w1_hbm, b1_hbm, w2_hbm, b2_hbm,
            out_hbm,
            wraw, woT, xT, w1, hT, w2, ostage, prev, prod, ws, wr, wsh, wn, prodn, wu, wz, prodz,
            yacc, act, uacc, xn, tt, ut, vt, zb, onat, hn, memc, bias2, mem0, b1_ref, b2_ref, xs0, zero,
            wsem, xsem, msem, osem):
    def raw_copy(n, w, p):
        return pltpu.make_async_copy(w.bitcast(U32).at[:, p, :], wraw.at[n, p], wsem.at[n, p])

    def qk_copies(p):
        return [raw_copy(0, wq_hbm, p), raw_copy(1, wk_hbm, p)]

    def vo_copies(p):
        heads = pl.ds(2 * p, 2)
        return [raw_copy(2, wv_hbm, p),
                pltpu.make_async_copy(woT_hbm.at[heads], woT.at[heads], wsem.at[3, p])]

    def x_copy(k):
        cols = (pl.ds(0, 128), pl.ds(128, 256), pl.ds(384, S - 384))[k]
        return pltpu.make_async_copy(xT_hbm.at[:, cols], xT.at[:, cols], xsem.at[k])

    def small_copies():
        pairs = ((mem_hbm, mem0), (b1_hbm, b1_ref), (b2_hbm, b2_ref))
        return [pltpu.make_async_copy(src, dst, xsem.at[3 + j]) for j, (src, dst) in enumerate(pairs)]

    def w1_copy():
        return pltpu.make_async_copy(w1_hbm, w1.at[pl.ds(256, S)], msem.at[0])

    def w2_copies():
        return [pltpu.make_async_copy(w2_hbm.at[:, pl.ds(YW * j, YW)], w2.at[j], msem.at[1 + j])
                for j in range(2 * YC)]

    def out_copy(q, c, part=0):
        rows, j = pl.ds(DH * (q // 2), DH), YC * (q % 2) + c
        w = YW // (LAST if q == 3 else 1)
        return pltpu.make_async_copy(ostage.at[j, rows, pl.ds(w * part, w)],
                                     out_hbm.at[rows, pl.ds(_aligned(j * (YW // w) + part, w), w)],
                                     osem.at[q + part, c])

    def head_pair(n, p):
        packed = wraw[n, p]
        even = pltpu.bitcast(packed << 16, F32)
        odd = pltpu.bitcast(packed & np.uint32(0xFFFF0000), F32)
        return even, odd

    def pair_products(l0, l1, r0, r1):
        l0, l1, r0, r1 = (v.astype(BF16) for v in (l0, l1, r0, r1))
        tail = jnp.concatenate([l0[DA:], l1[DA:]], axis=0)
        rest = [_dot_nt(r[DA:], jnp.concatenate([l[:DA], tail], axis=0)) for l, r in ((l0, r0), (l1, r1))]
        main = [_dot_nt(jnp.concatenate([l[DA:], l[:DA]], axis=0), r[:DA]) for l, r in ((l0, r0), (l1, r1))]
        return [(m[DB:], m[:DB]) for m in main], rest

    def store_weights(j, m0, m1, shared):
        quadrant = lambda q: (m0, m1)[q % 2][128 * (q // 2):128 * (q // 2 + 1)]
        for m in range(7):
            ws[j, m] = _words(_combine(quadrant, RIGHT[m]))
        wr[j] = _words(jnp.concatenate([m0[256:], m1[256:]], axis=1))
        wsh[j] = _words(shared[256:])
        prev[j] = shared[:256]

    def store_narrow(k):
        quadrant = lambda q: prev[2 * k + q % 2, 128 * (q // 2):128 * (q // 2 + 1), :]
        for m in range(7):
            wn[k, m] = _words(_combine(quadrant, RIGHT[m]))

    def token_factor(m, first, lo, hi):
        parts = []
        for r in range(lo, hi, 8):
            def load(q):
                row = first + 2 * SEG * (r // SEG) + SEG * (q // 2) + r % SEG
                return xn[pl.ds(row, 8), 128 * (q % 2):128 * (q % 2 + 1)]
            parts.append(_combine(load, LEFT[m]))
        return jnp.concatenate(parts, axis=0)

    def first_products(j):
        for m in range(7):
            x = xs0[m, 0:FIRST_ROWS[m], :]
            prod[j, pl.ds(BASE[m], FIRST_ROWS[m]), :] = _dot(x, pltpu.bitcast(ws[j, m], BF16))

    def absorb_qk(p):
        first_products(jnp.maximum(p - 1, 0))
        ((m0, t0), (m1, t1)), (r0, r1) = pair_products(*head_pair(0, p), *head_pair(1, p))
        shared = _transpose(jnp.concatenate([r0[:, :DA], r1[:, :DA]], axis=0))
        keyside = jnp.concatenate([_transpose(jnp.concatenate([t0, t1], axis=0)),
                                   jnp.where(_lanes(DB) < DB, r0[:, DA:], r1[:, DA:])], axis=0)
        wu[p] = _words(keyside[256:])
        prev[2 * NP + p] = keyside[:256]
        store_weights(p, m0, m1, shared)

    def absorb_vo(p):
        first_products(NP + p - 1)
        ((m0, t0), (m1, t1)), (r0, r1) = pair_products(*head_pair(2, p), woT[2 * p], woT[2 * p + 1])
        shared = _transpose(jnp.concatenate([r0, r1], axis=0))
        low = _lanes(DB) < DB
        z0 = jnp.concatenate([t0, jnp.where(low, shared[DA:D], 0.0)], axis=1)
        z1 = jnp.concatenate([t1, jnp.where(low, 0.0, shared[D:])], axis=1)
        pieces = [jnp.concatenate([_group(z0, dg), _group(z1, dg)], axis=0) for dg in range(DB // 8)]
        for dg in range(4):
            quadrant = lambda q: pieces[dg + 4 * (q // 2)][:, 256 * (q % 2):256 * (q % 2 + 1)]
            for m in range(7):
                wz[m, pl.ds(_aligned(8 * dg + p, 8), 8), :] = _words(_combine(quadrant, RIGHT[m]))
        store_weights(NP + p, m0, m1, shared[:DA])

    def absorb_all(copies, absorb):
        def body(p, carry):
            for c in copies(p):
                c.wait()
            absorb(p)
            return carry
        lax.fori_loop(0, NP, body, 0)

    def normalize_x(b, slot, mark=True):
        n = _layernorm(xT[:, pl.ds(_aligned(b, 128), 128)].astype(F32))
        n = jnp.concatenate([n, n[DA:]], axis=0)
        for c in range(DP // 128):
            tile = n[128 * c:128 * (c + 1)].T
            xn[pl.ds(128 * slot, 128), 128 * c:128 * (c + 1)] = tile
            if mark:
                hn[5, slot - 1, 8 * c:8 * (c + 1), :] = tile[120:]

    def put_pair(dst, even, odd, p):
        for g in range(NG):
            dst(g)[pl.ds(16 * p, 16), :] = jnp.concatenate(
                [_group(even, g), _group(odd, g)], axis=0).astype(BF16)

    def strassen_pass(factors, r, k, w_ref, saved, out):
        m, _, _, lo, hi = PASSES[r][k]
        t = _dot(factors[k], pltpu.bitcast(w_ref[m], BF16))
        out[m] = t[:M]
        for a in range(lo, hi, 8):
            saved[pl.ds(BASE[m] + (a + SEG) % RING[m], 8), :] = t[M + a - lo:M + a - lo + 8]

    def memory_terms(r, a):
        return sorted(((x[0], x[2][a]) for x in PASSES[r] if x[2][a]), key=lambda t: -t[1])

    def strassen_result(r, a, saved, out):
        terms = memory_terms(r, a)
        tokens = _merge(lambda m: saved[pl.ds(BASE[m] + SEG * (r // 2) % RING[m], SEG), :], MERGE[2 * (r % 2) + a])
        return jnp.concatenate([_merge(out.get, terms), tokens], axis=0)

    def attended_factor(m, lo, hi):
        parts = []
        for a in range(lo, hi, 8):
            row = (a + SEG) % (2 * SEG)
            load = lambda q: jnp.concatenate([zb[q // 2, 4 * (q % 2) + j, row:row + 8, :] for j in range(4)], axis=1)
            parts.append(_combine(load, LEFT[m]))
        return jnp.concatenate(parts, axis=0)

    def fold(o):
        ob = o[:, DA:]
        return jnp.concatenate([o[:, :DA], ob + pltpu.roll(ob, DB, 1)], axis=1)

    def complete_pair(k):
        for s_ in range(2):
            rows = pl.ds((2 * SEG * (k - 1) + SEG * s_) % 256, SEG)
            saved = lambda m: prodz[pl.ds(BASE[m] + SEG * (k + 1) % RING[m], SEG), :]
            late = jnp.concatenate([_merge(saved, MERGE[2 * s_ + a]) for a in range(2)], axis=1)
            onat[rows, :] = fold(onat[rows, :] + late)

    def put_masked(dst, t, p):
        low = _lanes(L) < DB
        put_pair(dst, jnp.where(low, t, 0.0), jnp.where(low, 0.0, t), p)

    def narrow(factors, r, k, rest, dst, p):
        out = {}
        for i in (0, 2, 1, 3):
            strassen_pass(factors, r, i, wn.at[k], prodn.at[k], out)
        for a in range(2):
            put_masked(dst, strassen_result(r, a, prodn.at[k], out) + rest(a), p + a)

    def project(h, factors, r, porder, first, dst, p):
        j, out = first + p, {}
        thirds = [None, None]
        for k in porder:
            if k == "R":
                t = _dot(h[:, 256:DA], pltpu.bitcast(wr[j], BF16))
                thirds = [t[:, :DA], t[:, DA:]]
            elif k in "ab":
                a = "ab".index(k)
                thirds[a] = _dot(h[:, 256:DA], pltpu.bitcast(wr[j, :, DA * a:DA * (a + 1)], BF16))
            elif k == "H":
                if p % 2:
                    rest = lambda a: _dot(h[:, 256:DA], pltpu.bitcast(wsh[j - 1 + a], BF16))
                    narrow(factors, r, j // 2, rest, lambda g: dst.at[g, 3], p - 1)
            else:
                strassen_pass(factors, r, int(k), ws.at[j], prod.at[j], out)
        heads = [strassen_result(r, a, prod.at[j], out) + thirds[a] for a in range(2)]
        for c in range(3):
            put_pair(lambda g: dst.at[g, c], heads[0][:, 128 * c:128 * (c + 1)], heads[1][:, 128 * c:128 * (c + 1)], p)

    def step(mem, r, mix):
        h = jnp.concatenate([mem, xn[pl.ds(SEG * r, SEG), :]], axis=0)
        hb = h[:, DA:]
        hbT = jnp.concatenate([hb, jnp.zeros((128 - L, 128), F32)], axis=0).T[:DB]
        halves = {M1: mem[:, :128], M2: mem[:, 128:256], M12: mem[:, :128] + mem[:, 128:256]}
        factors = [jnp.concatenate([halves[mix_], token_factor(m, 2 * SEG, lo, hi)], axis=0)
                   for m, mix_, _, lo, hi in PASSES[r]]
        cross, direct, probs, weights = {}, {}, {}, {}
        rows = [None] * NG

        def accumulate(g, v):
            rows[g] = v if rows[g] is None else rows[g] + v

        def key_side(k):
            rest = lambda a: _dot(h[:, 256:D], pltpu.bitcast(wu[2 * k + a], BF16))
            narrow(factors, r, 8 + k, rest, lambda g: ut.at[g], 2 * k)

        def cross_scores(gk):
            gqs = [gq for gq in range(NG) if _visible(gq, gk)]
            s = _dot_nt(jnp.concatenate([_group(hb, gq) for gq in gqs], axis=0), ut[gk])
            for i, gq in enumerate(gqs):
                cross[gq, gk] = _swap8(_group(s, i))

        def direct_scores(gq):
            n = sum(_visible(gq, gk) for gk in range(NG))
            queries = jnp.concatenate([tt[gq, c] for c in range(4)], axis=1)
            direct[gq] = _dot_nt(h[:8 * n], queries)

        def softmax(gq):
            n = direct[gq].shape[0] // 8
            parts = []
            for gk in range(n):
                s = _group(direct[gq], gk) + cross[gq, gk]
                if gq > 0 and gk == gq:
                    s = jnp.where(_sublanes() <= (_lanes(8) & 7), s, -1e9 / SCALE)
                parts.append(s)
            s = jnp.concatenate(parts, axis=0)
            e = jnp.exp2((s - jnp.max(s, axis=0, keepdims=True)) * (SCALE * LOG2E))
            pt = e * (1.0 / jnp.sum(e, axis=0, keepdims=True))
            for gk in range(n):
                probs[gq, gk] = _swap8(_group(pt, gk))
            if n % 2:
                pt = jnp.concatenate([pt, jnp.zeros((8, 128), F32)], axis=0)
            weights[gq] = pt.astype(BF16)

        def attend(gq):
            zT = _dot(hbT[:, :weights[gq].shape[0]], weights[gq])
            for dg in range(DB // 8):
                slot, row = (r % 2, SEG * (r // 2 % 2) + 8 * (gq - 1)) if gq else (2, 0)
                zb[slot, dg, row:row + 8, :] = _swap8(_group(zT, dg))

        late = {}

        def late_values(k):
            m, halves_, _, lo, hi = PASSES[r][k]
            slot = 2 if late else 2 + zero[0]
            half = lambda a: jnp.concatenate([zb[slot, 4 * a + j, 0:M, :] for j in range(4)], axis=1)
            own = half(0) + half(1) if halves_ == M12 else half(halves_[1])
            factor = jnp.concatenate([own, attended_factor(m, lo, hi)], axis=0)
            strassen_pass({k: factor}, r, k, wz, prodz, late)

        def early_values(gk):
            gqs = [gq for gq in range(NG) if _visible(gq, gk)]
            values = jnp.concatenate([vt[gk, c] for c in range(4)], axis=1)
            part = _dot(jnp.concatenate([probs[gq, gk] for gq in gqs], axis=0), values)
            for i, gq in enumerate(gqs):
                accumulate(gq, _group(part, i))

        pieces = dict(U=key_side, T=functools.partial(project, h, factors, r, PROJECT_ORDER[r][0], 0, tt),
                      V=functools.partial(project, h, factors, r, PROJECT_ORDER[r][1], NP, vt), C=cross_scores, D=direct_scores,
                      X=softmax, Z=attend, A=late_values, P=early_values, M=mix)
        for name, index in STEP_ORDER[r].split():
            pieces[name](int(index))
        own = jnp.concatenate([_merge(late.get, memory_terms(r, a)) for a in range(2)], axis=1)
        return fold(rows[0] + own), jnp.concatenate(rows[1:], axis=0)

    def finish_block(b, half):
        oT = _transpose(onat[128 * half:128 * (half + 1), :])
        cols = pl.ds(_aligned(b if isinstance(b, int) else jnp.maximum(b, 0), 128), 128)
        res = xT[:, cols].astype(F32) + oT[:D]
        hT[b + 1] = res
        hn[3 + half, 0] = res[:DH]
        hn[3 + half, 1] = res[DH:]

    def normalize_block(half, slot):
        n = _double_layernorm(jnp.concatenate([hn[3 + half, 0], hn[3 + half, 1]], axis=0))
        hn[slot, 0] = n[:DH]
        hn[slot, 1] = n[DH:]

    def mix_unit(i, m, n, parts=1, pin=False):
        def load(q):
            return w1[pl.ds(_aligned(2 * i + 2 + q // 2, 128), 128), pl.ds(FH * (q % 2) + 128 * n, 128)]
        cols = pl.ds(128 * n, 128)
        w = _combine(load, RIGHT[m]).astype(BF16)
        for k in range(parts):
            rows = pl.ds(DH // parts * k, DH // parts)
            x = _combine(lambda q: hn[q % 2 + zero[0] if pin else q % 2, q // 2, rows, :], LEFT[m])
            total = uacc[m, rows, cols] + _dot(x, w)
            uacc[m, rows, cols] = total if isinstance(i, int) else jnp.where(i >= 0, total, 0.0)

    def iteration(i):
        chores = dict(F=lambda: finish_block(2 * i - 1, 1), L=lambda: normalize_block(1, 1),
                      f=lambda: finish_block(2 * i, 0), l=lambda: normalize_block(0, 2),
                      N=lambda: normalize_x(2 * i + 1, 1), n=lambda: normalize_x(2 * i + 2, 2))
        xn[0:128, :] = xn[256:384, :]
        hn[0] = hn[2]
        mem = memc[...]
        for r in range(8):
            for name in CHORES[r]:
                chores[name]()

            def mix(part, r=r):
                split, parts = MIX_SPLIT[r]
                lo = 6 * r + sum(split[:part])
                hi = lo + split[part] + (r == 7 and part == len(split) - 1)
                for m, n in MIX_UNITS[lo:hi]:
                    mix_unit(i - 1, m, n, parts[part], (r, part) in PINS)
            mem, o = step(mem, r, mix)
            onat[SEG * r:SEG * (r + 1), :] = o
            if r % 2:
                complete_pair(r // 2)
        memc[...] = mem

    def activate(q, lo, hi):
        cols = pl.ds(128 * lo, 128 * (hi - lo))
        first = FH * (q % 2) + 128 * lo
        b1 = b1_ref[...].astype(F32).reshape(1, F)[:, first:first + 128 * (hi - lo)]
        u = _merge(lambda m: uacc[m, :, cols], MERGE[q]) + b1
        t = jnp.tanh(u * (GELU_C + (GELU_C * 0.044715) * (u * u)))
        half = 0.5 * u
        act[q, :, cols] = half + half * t

    def project_out(m, c, lo, hi, cols=slice(None)):
        def load(q):
            return w2[YC * (q % 2) + c, pl.ds(FH * (q // 2) + 128 * lo, 128 * (hi - lo)), cols]
        x = _combine(lambda q: act[q, :, pl.ds(128 * lo, 128 * (hi - lo))], LEFT[m])
        y = _dot(x, _combine(load, RIGHT[m]).astype(BF16))
        yacc[m, c, :, cols] = y if lo == 0 else yacc[m, c, :, cols] + y

    def emit(q, c, part=0):
        rows, j = pl.ds(DH * (q // 2), DH), YC * (q % 2) + c
        w = YW // (LAST if q == 3 else 1)
        cols = pl.ds(w * part, w)
        first = j * (YW // 128) + part * (w // 128) + 1
        res = jnp.concatenate([hT[first + k, rows, :] for k in range(w // 128)], axis=1)
        y = _merge(lambda m: yacc[m, c, :, cols], MERGE[q])
        ostage[j, rows, cols] = (res + y + bias2[j, :, cols]).astype(BF16)
        out_copy(q, c, part).start()

    def run_tail(order, chunks):
        for name, index in order.split():
            i = int(index)
            lo, hi = (0, 1) if name.islower() else (1, FT)
            if name == "N":
                for m, n in MIX_UNITS[:2 * FT]:
                    mix_unit(NI - 1, m, n)
            elif name == "M":
                for m in (0, 1, 3, 4, 6):
                    mix_unit(NI - 1, m, i)
            elif name in "gG":
                activate(i, lo, hi)
            for c in chunks:
                if name in "yY":
                    project_out(i, c, lo, hi)
                elif name == "E":
                    emit(i, c)
                elif name == "Z":
                    for part in range(LAST):
                        project_out(i, c, lo, hi, pl.ds(YW // LAST * part, YW // LAST))
                        emit(3, c, part)

    def tail():
        for c in w2_copies():
            c.wait()
        for m in range(7):
            lo = FIRST_ROWS[m] - SEG
            prodz[pl.ds(BASE[m] + (SEG + lo) % RING[m], SEG - lo), :] = _dot(attended_factor(m, lo, SEG), pltpu.bitcast(wz[m], BF16))
        complete_pair(0)
        finish_block(NB - 1, 1)
        hn[0] = hn[2]
        normalize_block(1, 1)
        run_tail(TAIL_HEAD, range(YC))

        def chunk(c, carry):
            run_tail(TAIL_BODY, [c])
            return carry
        lax.fori_loop(0, YC, chunk, 0)
        for c in range(YC):
            for q in range(3):
                out_copy(q, c).wait()
            for part in range(LAST):
                out_copy(3, c, part).wait()

    zero[0] = 0

    def prologue():
        for c in small_copies():
            c.start()
        x_copy(0).start()
        for copies in (qk_copies, vo_copies):
            def start(p, carry, copies=copies):
                for c in copies(p):
                    c.start()
                return carry
            lax.fori_loop(0, NP, start, 0)
        x_copy(1).start()
        for c in small_copies():
            c.wait()
        m0 = mem0[0].astype(F32)
        memc[...] = jnp.concatenate([m0, m0[:, DA:]], axis=1)
        b2 = b2_ref[...].astype(F32).reshape(1, S)
        for j in range(2 * YC):
            bias2[j] = b2[:, YW * j:YW * (j + 1)]
        x_copy(0).wait()
        normalize_x(0, 2, False)
        for m in range(7):
            xs0[m, 0:FIRST_ROWS[m], :] = token_factor(m, 256, 0, FIRST_ROWS[m])
        absorb_all(qk_copies, absorb_qk)
        absorb_all(vo_copies, absorb_vo)
        first_products(2 * NP - 1)
        for k in range(12):
            store_narrow(k)
            for m in range(7):
                rows = FIRST_ROWS[m]
                prodn[k, pl.ds(BASE[m], rows), :] = _dot(xs0[m, 0:rows, :], pltpu.bitcast(wn[k, m], BF16))
        x_copy(1).wait()
        x_copy(2).start()
        w1_copy().start()
        for c in w2_copies():
            c.start()

    def body(t, carry):
        pl.when(t == 0)(prologue)

        @pl.when(jnp.logical_and(t >= 1, t <= NI))
        def _():
            i = jnp.clip(t - 1, 0, NI - 1)

            @pl.when(i == 1)
            def _():
                x_copy(2).wait()
                w1_copy().wait()
            iteration(i)

        pl.when(t == NI + 1)(tail)
        return carry

    lax.fori_loop(0, NI + 2, body, 0)


@functools.partial(jax.jit, static_argnames=("A_seg_len",))
def pallas_sequential_preLN__memory_aug_recurrent_mem_tr__mixer_token_mlp__prompt_kernel(
    A_x: jax.Array,
    A_mem0: jax.Array,
    A_Wq: jax.Array,
    A_Wk: jax.Array,
    A_Wv: jax.Array,
    A_Wo: jax.Array,
    A_seg_len: int,
    B_x: jax.Array,
    B_w1: jax.Array,
    B_b1: jax.Array,
    B_w2: jax.Array,
    B_b2: jax.Array,
):
    del B_x
    assert A_seg_len == SEG and A_x.shape == (1, S, D) and A_mem0.shape == (1, M, D)
    assert A_Wq.shape == (D, H, E) and A_Wo.shape == (H, E, D) and B_w1.shape == (S, F)
    hbm = pl.BlockSpec(memory_space=pl.ANY)
    out = pl.pallas_call(
        _kernel,
        out_shape=jax.ShapeDtypeStruct((D, S), BF16),
        in_specs=[hbm] * 10,
        out_specs=hbm,
        scratch_shapes=[
            pltpu.VMEM((3, NP, D, E), U32),
            pltpu.VMEM((H, D, E), BF16),
            pltpu.VMEM((D, S + 128), BF16),
            pltpu.VMEM((S + 256, F), BF16),
            pltpu.VMEM((NB + 1, D, 128), F32),
            pltpu.VMEM((2 * YC, F, YW), BF16),
            pltpu.VMEM((2 * YC, D, YW), BF16),
            pltpu.VMEM((3 * NP, 256, 128), F32),
            pltpu.VMEM((2 * NP, SAVED, DA), F32),
            pltpu.VMEM((2 * NP, 7, 64, DA), U32),
            pltpu.VMEM((2 * NP, 64, 2 * DA), U32),
            pltpu.VMEM((2 * NP, 64, 128), U32),
            pltpu.VMEM((12, 7, 64, 128), U32),
            pltpu.VMEM((12, SAVED, 128), F32),
            pltpu.VMEM((NP, (D - 256) // 2, 128), U32),
            pltpu.VMEM((7, 256, DP // 2), U32),
            pltpu.VMEM((SAVED, DP // 2), F32),
            pltpu.VMEM((7, YC, DH, YW), F32),
            pltpu.VMEM((4, DH, FH), F32),
            pltpu.VMEM((7, DH, FH), F32),
            pltpu.VMEM((384, DP), F32),
            pltpu.VMEM((NG, 4, 128, 128), BF16),
            pltpu.VMEM((NG, 128, 128), BF16),
            pltpu.VMEM((NG, 4, 128, 128), BF16),
            pltpu.VMEM((3, DB // 8, 64, 128), F32),
            pltpu.VMEM((256, DP), F32),
            pltpu.VMEM((6, 2, DH, 128), F32),
            pltpu.VMEM((M, DP), F32),
            pltpu.VMEM((2 * YC, 1, YW), F32),
            pltpu.VMEM((1, M, D), BF16),
            pltpu.VMEM((F,), BF16),
            pltpu.VMEM((S,), BF16),
            pltpu.VMEM((7, 48, 128), F32),
            pltpu.SMEM((1,), jnp.int32),
            pltpu.SemaphoreType.DMA((4, NP)),
            pltpu.SemaphoreType.DMA((6,)),
            pltpu.SemaphoreType.DMA((1 + 2 * YC,)),
            pltpu.SemaphoreType.DMA((3 + LAST, YC)),
        ],
        compiler_params=pltpu.CompilerParams(vmem_limit_bytes=120 * 2 ** 20),
        name="rmt_mixer",
    )(
        jnp.transpose(A_x, (0, 2, 1)).reshape(D, S),
        A_mem0, A_Wq, A_Wk, A_Wv,
        jnp.transpose(A_Wo, (0, 2, 1)),
        B_w1, B_b1, B_w2, B_b2,
    )
    return jnp.transpose(out.reshape(1, D, S), (0, 2, 1))
```
